```python
import os as _os
_os.environ.setdefault("JAX_PLATFORMS", "cpu")
import jax
import jax.numpy as jnp

def _softmax(x, axis=-1):
    return jax.nn.softmax(x, axis=axis)
def _gelu(x):
    return jax.nn.gelu(x, approximate=True)
def _silu(x):
    return jax.nn.silu(x)
def _sigmoid(x):
    return jax.nn.sigmoid(x)
def _layernorm(x, axis=-1, eps=1e-5):
    m = jnp.mean(x, axis=axis, keepdims=True)
    v = jnp.var(x, axis=axis, keepdims=True)
    return (x - m) / jnp.sqrt(v + eps)
def _scatter_add(tgt, idx, src, axis=0):
    return tgt.at[idx].add(src)
def _segment_sum(src, seg, n):
    return jax.ops.segment_sum(src, seg, n)
class _Rng:
    def __init__(self, key):
        self._k = key
    def _next(self):
        self._k, sub = jax.random.split(self._k)
        return sub
    def normal(self, shape):
        return jax.random.normal(self._next(), shape, dtype=jnp.bfloat16)
    def randint(self, lo, hi, shape):
        return jax.random.randint(self._next(), shape, lo, hi, dtype=jnp.int32)
    def uniform(self, shape, lo=0.0, hi=1.0):
        return jax.random.uniform(self._next(), shape, jnp.bfloat16, lo, hi)
    def permutation(self, n):
        return jax.random.permutation(self._next(), n)


kernel_name = 'sequential_preLN__mha_block__moe_arch_mod__prompt'

def setup_inputs():
    _rng = _Rng(jax.random.key(int.from_bytes(__import__("os").urandom(4), "little")))
    _w = (lambda a: (lambda t: t.astype(jnp.bfloat16) if jnp.issubdtype(t.dtype, jnp.floating) else t)(jnp.asarray(a)))
    def _A_setup():
        B, S, D, H = 1, 2048, 640, 32
        return {
            "x": _w((lambda *s: _rng.normal(s) * 0.05)(B, S, D)),
            "wqkv": _w((lambda *s: _rng.normal(s) * 0.05)(D, 3 * D)),
            "wo": _w((lambda *s: _rng.normal(s) * 0.05)(D, D)),
        }
    _A_in = _A_setup()

    def _B_setup():
        B, S, D, F, C = 1, 2048, 640, 1536, 1
        return {
            "x": _w((lambda *s: _rng.normal(s) * 0.05)(B, S, D)),
            "w_r": _w((lambda *s: _rng.normal(s) * 0.05)(D)),
            "w_gate": _w((lambda *s: _rng.normal(s) * 0.05)(D, F)),
            "w_up": _w((lambda *s: _rng.normal(s) * 0.05)(D, F)),
            "w_down": _w((lambda *s: _rng.normal(s) * 0.05)(F, D)),
        }
    _B_in = _B_setup()

    return {
        "A_x": _A_in["x"],
        "A_wqkv": _A_in["wqkv"],
        "A_wo": _A_in["wo"],
        "B_x": _B_in["x"],
        "B_w_r": _B_in["w_r"],
        "B_w_gate": _B_in["w_gate"],
        "B_w_up": _B_in["w_up"],
        "B_w_down": _B_in["w_down"],
    }

def reference(A_x, A_wqkv, A_wo, B_x, B_w_r, B_w_gate, B_w_up, B_w_down):
    def _A_ref(x, wqkv, wo):
        B, S, D = x.shape
        H = 32
        Dh = D // H
        qkv = (lambda x, *d: x.transpose(*d))((x @ wqkv).reshape(B, S, 3, H, Dh), 2, 0, 3, 1, 4)
        q, k, v = qkv[0], qkv[1], qkv[2]
        scores = jnp.einsum("bhqd,bhkd->bhqk", q, k) * (Dh ** -0.5)
        p = _softmax(scores, axis=-1)
        o = jnp.einsum("bhqk,bhkd->bhqd", p, v)
        return (lambda x, *d: x.transpose(*d))(o, 0, 2, 1, 3).reshape(B, S, D) @ wo

    def _B_ref(x, w_r, w_gate, w_up, w_down):
        B, S, D = x.shape
        C = 1
        r = x @ w_r
        idx = jnp.argsort(-r, axis=-1)[:, :C]
        idx_e = jnp.repeat(idx.reshape(B, C, 1), D, axis=2)
        x_sel = jnp.take_along_axis(x, idx_e, axis=1)
        g = _silu(x_sel @ w_gate)
        u = x_sel @ w_up
        y = (g * u) @ w_down
        r_sel = _sigmoid(jnp.take_along_axis(r, idx, axis=1))
        y = y * r_sel.reshape(B, C, 1)
        b_off = (jnp.arange(B) * S).reshape(B, 1)
        flat_idx = (idx + b_off).reshape(B * C)
        zero = (x * 0.0).reshape(B * S, D)
        upd = _scatter_add(zero, flat_idx, y.reshape(B * C, D), axis=0)
        return x + upd.reshape(B, S, D)

    x = A_x
    h = x + _A_ref(_layernorm(x, axis=-1), A_wqkv, A_wo)
    h2 = h + _B_ref(_layernorm(h, axis=-1), B_w_r, B_w_gate, B_w_up, B_w_down)
    return h2
```

```python
import jax
import jax.numpy as jnp
import jax.experimental.pallas as pl
import jax.experimental.pallas.tpu as pltpu

S = 2048
D = 640
H = 32
DH = 20
HP = 32
NG = H * HP // 128
F = 1536
TQ = 512
RC = 256
EPS = 1e-5
ONES_LANE = DH


def _ln(x):
    m = jnp.mean(x, axis=-1, keepdims=True)
    xc = x - m
    v = jnp.mean(xc * xc, axis=-1, keepdims=True)
    return xc * jax.lax.rsqrt(v + EPS)


def _kernel(x_ref, wqkv_ref, wo_ref, wr_ref, wg_ref, wu_ref, wd_ref, o_ref,
            q_s, kT_s, v_s, on_s, lnh_s):
    f32 = jnp.float32
    bf16 = jnp.bfloat16
    scale = DH ** -0.5

    lane128 = jax.lax.broadcasted_iota(jnp.int32, (1, 128), 1)
    ones_mask = (lane128 % HP) == ONES_LANE

    def p1(c, carry):
        r0 = pl.multiple_of(c * RC, RC)
        xs = x_ref[pl.ds(r0, RC), :].astype(f32)
        ln = _ln(xs).astype(bf16)
        for g in range(NG):
            q = jnp.dot(ln, wqkv_ref[:, g * 128:(g + 1) * 128], preferred_element_type=f32)
            q_s[g, pl.ds(r0, RC), :] = (q * scale).astype(bf16)
            k = jnp.dot(ln, wqkv_ref[:, 1024 + g * 128:1024 + (g + 1) * 128],
                        preferred_element_type=f32)
            kT_s[g, :, pl.ds(r0, RC)] = k.T.astype(bf16)
            v = jnp.dot(ln, wqkv_ref[:, 2048 + g * 128:2048 + (g + 1) * 128],
                        preferred_element_type=f32)
            v = jnp.where(ones_mask, 1.0, v)
            v_s[g, pl.ds(r0, RC), :] = v.astype(bf16)
        return carry

    jax.lax.fori_loop(0, S // RC, p1, 0)

    er = jax.lax.broadcasted_iota(jnp.int32, (128, 128), 0)
    ec = jax.lax.broadcasted_iota(jnp.int32, (128, 128), 1)
    E = jnp.where((er % HP == ONES_LANE) & (er // HP == ec // HP), 1.0, 0.0).astype(f32)

    def p2(i, carry):
        qb = i // NG
        g = i % NG
        r0 = pl.multiple_of(qb * TQ, TQ)
        qg = q_s[g, pl.ds(r0, TQ), :]
        kT = kT_s[g]
        vg = v_s[g]
        acc = jnp.zeros((TQ, 128), f32)
        for j in range(4):
            hmask = (lane128 // HP) == j
            qm = jnp.where(hmask, qg, jnp.zeros_like(qg))
            s = jnp.dot(qm, kT, preferred_element_type=f32)
            m = jnp.max(s, axis=-1, keepdims=True)
            p = jnp.exp(s - m).astype(bf16)
            o = jnp.dot(p, vg, preferred_element_type=f32)
            acc = jnp.where(hmask, o, acc)
        l = jnp.dot(acc, E, preferred_element_type=f32, precision=jax.lax.Precision.HIGHEST)
        on_s[g, pl.ds(r0, TQ), :] = (acc / l).astype(bf16)
        return carry

    jax.lax.fori_loop(0, (S // TQ) * NG, p2, 0)

    wr = wr_ref[...].astype(f32)

    def p3(c, carry):
        best_v, best_i = carry
        r0 = pl.multiple_of(c * RC, RC)
        a = jnp.zeros((RC, D), f32)
        for g in range(NG):
            a = a + jnp.dot(on_s[g, pl.ds(r0, RC), :], wo_ref[g * 128:(g + 1) * 128, :],
                            preferred_element_type=f32)
        a = a.astype(bf16).astype(f32)
        xs = x_ref[pl.ds(r0, RC), :].astype(f32)
        h = (xs + a).astype(bf16).astype(f32)
        lnh = _ln(h).astype(bf16).astype(f32)
        lnh_s[pl.ds(r0, RC), :] = lnh
        o_ref[pl.ds(r0, RC), :] = (h + lnh).astype(o_ref.dtype)
        r = jnp.sum(lnh * wr, axis=-1, keepdims=True)
        r = r.astype(bf16).astype(f32)
        cm = jnp.max(r)
        rows = jax.lax.broadcasted_iota(jnp.int32, (RC, 1), 0) + c * RC
        ci = jnp.min(jnp.where(r == cm, rows, S))
        better = cm > best_v
        return jnp.where(better, cm, best_v), jnp.where(better, ci, best_i)

    best_v, best_i = jax.lax.fori_loop(
        0, S // RC, p3, (jnp.float32(-jnp.inf), jnp.int32(0)))

    xsel = lnh_s[pl.ds(best_i, 1), :]
    xsel8 = jnp.broadcast_to(xsel, (8, D)).astype(bf16)
    gt = jnp.dot(xsel8, wg_ref[...], preferred_element_type=f32)
    gt = gt.astype(bf16).astype(f32)
    gt = (gt * jax.nn.sigmoid(gt)).astype(bf16).astype(f32)
    u = jnp.dot(xsel8, wu_ref[...], preferred_element_type=f32).astype(bf16).astype(f32)
    gu = (gt * u).astype(bf16)
    y = jnp.dot(gu, wd_ref[...], preferred_element_type=f32).astype(bf16).astype(f32)
    rs = jax.nn.sigmoid(best_v).astype(bf16).astype(f32)
    y = (y * rs).astype(bf16).astype(f32)
    t0 = pl.multiple_of((best_i // 16) * 16, 16)
    rows = jax.lax.broadcasted_iota(jnp.int32, (16, 1), 0) + t0
    cur = o_ref[pl.ds(t0, 16), :].astype(f32)
    y16 = jnp.broadcast_to(y[0:1, :], (16, D))
    o_ref[pl.ds(t0, 16), :] = jnp.where(rows == best_i, cur + y16, cur).astype(o_ref.dtype)


@jax.jit
def pallas_sequential_preLN__mha_block__moe_arch_mod__prompt_kernel(
    A_x: jax.Array,
    A_wqkv: jax.Array,
    A_wo: jax.Array,
    B_x: jax.Array,
    B_w_r: jax.Array,
    B_w_gate: jax.Array,
    B_w_up: jax.Array,
    B_w_down: jax.Array,
):
    del B_x
    x = A_x.reshape(S, D)
    wqkv = jnp.pad(A_wqkv.reshape(D, 3, H, DH), ((0, 0), (0, 0), (0, 0), (0, HP - DH)))
    wqkv = wqkv.reshape(D, 3 * H * HP)
    wo = jnp.pad(A_wo.reshape(H, DH, D), ((0, 0), (0, HP - DH), (0, 0))).reshape(H * HP, D)
    wr = B_w_r.reshape(1, D)

    vm = pl.BlockSpec(memory_space=pltpu.VMEM)
    out = pl.pallas_call(
        _kernel,
        out_shape=jax.ShapeDtypeStruct((S, D), A_x.dtype),
        in_specs=[vm] * 7,
        out_specs=vm,
        scratch_shapes=[
            pltpu.VMEM((NG, S, 128), jnp.bfloat16),
            pltpu.VMEM((NG, 128, S), jnp.bfloat16),
            pltpu.VMEM((NG, S, 128), jnp.bfloat16),
            pltpu.VMEM((NG, S, 128), jnp.bfloat16),
            pltpu.VMEM((S, D), jnp.float32),
        ],
        compiler_params=pltpu.CompilerParams(vmem_limit_bytes=100 * 1024 * 1024),
    )(x, wqkv, wo, wr, B_w_gate, B_w_up, B_w_down)
    return out.reshape(1, S, D)
```

```python
import jax
import jax.numpy as jnp
import jax.experimental.pallas as pl
import jax.experimental.pallas.tpu as pltpu

S = 2048
D = 640
H = 32
DH = 20
HP = 32
NG = H * HP // 128
F = 1536
TQ = 512
RC = 256
EPS = 1e-5
ONES_LANE = DH


def _ln(x):
    m = jnp.mean(x, axis=-1, keepdims=True)
    xc = x - m
    v = jnp.mean(xc * xc, axis=-1, keepdims=True)
    return xc * jax.lax.rsqrt(v + EPS)


def _kernel(x_ref, wqkv_ref, wo_ref, wr_ref, wg_hbm, wu_hbm, wd_hbm, o_ref,
            q_s, kT_s, v_s, on_s, lnh_s, wop_s, wg_ref, wu_ref, wd_ref, sems):
    f32 = jnp.float32
    bf16 = jnp.bfloat16
    scale = DH ** -0.5

    lane128 = jax.lax.broadcasted_iota(jnp.int32, (1, 128), 1)
    ones_mask = (lane128 % HP) == ONES_LANE

    cps = [pltpu.make_async_copy(wg_hbm, wg_ref, sems.at[0]),
           pltpu.make_async_copy(wu_hbm, wu_ref, sems.at[1]),
           pltpu.make_async_copy(wd_hbm, wd_ref, sems.at[2])]
    for cp in cps:
        cp.start()

    for hh in range(H):
        wop_s[hh * HP:hh * HP + DH, :] = wo_ref[hh * DH:(hh + 1) * DH, :].astype(f32)
        wop_s[hh * HP + DH:(hh + 1) * HP, :] = jnp.zeros((HP - DH, D), f32)

    zpad_l = jnp.zeros((RC, HP - DH), f32)
    lane_p = jax.lax.broadcasted_iota(jnp.int32, (RC, HP - DH), 1)
    one_pad = jnp.where(lane_p == 0, 1.0, 0.0).astype(f32)
    zpad_r = jnp.zeros((HP - DH, RC), f32)

    def p1(c, carry):
        r0 = pl.multiple_of(c * RC, RC)
        xs = x_ref[pl.ds(r0, RC), :].astype(f32)
        ln = _ln(xs).astype(bf16)
        q = jnp.dot(ln, wqkv_ref[:, 0:D], preferred_element_type=f32) * scale
        k = jnp.dot(ln, wqkv_ref[:, D:2 * D], preferred_element_type=f32)
        v = jnp.dot(ln, wqkv_ref[:, 2 * D:3 * D], preferred_element_type=f32)
        kt = k.T
        for g in range(NG):
            qp, kp, vp = [], [], []
            for j in range(4):
                hh = g * 4 + j
                qp += [q[:, hh * DH:(hh + 1) * DH], zpad_l]
                vp += [v[:, hh * DH:(hh + 1) * DH], one_pad]
                kp += [kt[hh * DH:(hh + 1) * DH, :], zpad_r]
            q_s[g, pl.ds(r0, RC), :] = jnp.concatenate(qp, axis=1).astype(bf16)
            v_s[g, pl.ds(r0, RC), :] = jnp.concatenate(vp, axis=1).astype(bf16)
            kT_s[g, :, pl.ds(r0, RC)] = jnp.concatenate(kp, axis=0).astype(bf16)
        return carry

    jax.lax.fori_loop(0, S // RC, p1, 0)

    er = jax.lax.broadcasted_iota(jnp.int32, (128, 128), 0)
    ec = jax.lax.broadcasted_iota(jnp.int32, (128, 128), 1)
    E = jnp.where((er % HP == ONES_LANE) & (er // HP == ec // HP), 1.0, 0.0).astype(f32)

    def p2(i, carry):
        qb = i // NG
        g = i % NG
        r0 = pl.multiple_of(qb * TQ, TQ)
        qg = q_s[g, pl.ds(r0, TQ), :]
        kT = kT_s[g]
        vg = v_s[g]
        acc = jnp.zeros((TQ, 128), f32)
        for j in range(4):
            hmask = (lane128 // HP) == j
            qm = jnp.where(hmask, qg, jnp.zeros_like(qg))
            s = jnp.dot(qm, kT, preferred_element_type=f32)
            m = jnp.max(s, axis=-1, keepdims=True)
            p = jnp.exp(s - m).astype(bf16)
            o = jnp.dot(p, vg, preferred_element_type=f32)
            acc = jnp.where(hmask, o, acc)
        l = jnp.dot(acc, E, preferred_element_type=f32, precision=jax.lax.Precision.HIGHEST)
        on_s[g, pl.ds(r0, TQ), :] = (acc / l).astype(bf16)
        return carry

    jax.lax.fori_loop(0, (S // TQ) * NG, p2, 0)

    wr = wr_ref[...].astype(f32)

    def p3(c, carry):
        best_v, best_i = carry
        r0 = pl.multiple_of(c * RC, RC)
        a = jnp.zeros((RC, D), f32)
        for g in range(NG):
            a = a + jnp.dot(on_s[g, pl.ds(r0, RC), :], wop_s[g * 128:(g + 1) * 128, :].astype(bf16),
                            preferred_element_type=f32)
        a = a.astype(bf16).astype(f32)
        xs = x_ref[pl.ds(r0, RC), :].astype(f32)
        h = (xs + a).astype(bf16).astype(f32)
        lnh = _ln(h).astype(bf16).astype(f32)
        lnh_s[pl.ds(r0, RC), :] = lnh
        o_ref[pl.ds(r0, RC), :] = (h + lnh).astype(o_ref.dtype)
        r = jnp.sum(lnh * wr, axis=-1, keepdims=True)
        r = r.astype(bf16).astype(f32)
        cm = jnp.max(r)
        rows = jax.lax.broadcasted_iota(jnp.int32, (RC, 1), 0) + c * RC
        ci = jnp.min(jnp.where(r == cm, rows, S))
        better = cm > best_v
        return jnp.where(better, cm, best_v), jnp.where(better, ci, best_i)

    best_v, best_i = jax.lax.fori_loop(
        0, S // RC, p3, (jnp.float32(-jnp.inf), jnp.int32(0)))

    for cp in cps:
        cp.wait()
    xsel = lnh_s[pl.ds(best_i, 1), :]
    xsel8 = jnp.broadcast_to(xsel, (8, D)).astype(bf16)
    gt = jnp.dot(xsel8, wg_ref[...], preferred_element_type=f32)
    gt = gt.astype(bf16).astype(f32)
    gt = (gt * jax.nn.sigmoid(gt)).astype(bf16).astype(f32)
    u = jnp.dot(xsel8, wu_ref[...], preferred_element_type=f32).astype(bf16).astype(f32)
    gu = (gt * u).astype(bf16)
    y = jnp.dot(gu, wd_ref[...], preferred_element_type=f32).astype(bf16).astype(f32)
    rs = jax.nn.sigmoid(best_v).astype(bf16).astype(f32)
    y = (y * rs).astype(bf16).astype(f32)
    t0 = pl.multiple_of((best_i // 16) * 16, 16)
    rows = jax.lax.broadcasted_iota(jnp.int32, (16, 1), 0) + t0
    cur = o_ref[pl.ds(t0, 16), :].astype(f32)
    y16 = jnp.broadcast_to(y[0:1, :], (16, D))
    o_ref[pl.ds(t0, 16), :] = jnp.where(rows == best_i, cur + y16, cur).astype(o_ref.dtype)


@jax.jit
def pallas_sequential_preLN__mha_block__moe_arch_mod__prompt_kernel(
    A_x: jax.Array,
    A_wqkv: jax.Array,
    A_wo: jax.Array,
    B_x: jax.Array,
    B_w_r: jax.Array,
    B_w_gate: jax.Array,
    B_w_up: jax.Array,
    B_w_down: jax.Array,
):
    del B_x
    x = A_x.reshape(S, D)
    wqkv = A_wqkv
    wo = A_wo
    wr = B_w_r.reshape(1, D)

    vm = pl.BlockSpec(memory_space=pltpu.VMEM)
    out = pl.pallas_call(
        _kernel,
        out_shape=jax.ShapeDtypeStruct((S, D), A_x.dtype),
        in_specs=[vm] * 4 + [pl.BlockSpec(memory_space=pl.ANY)] * 3,
        out_specs=vm,
        scratch_shapes=[
            pltpu.VMEM((NG, S, 128), jnp.bfloat16),
            pltpu.VMEM((NG, 128, S), jnp.bfloat16),
            pltpu.VMEM((NG, S, 128), jnp.bfloat16),
            pltpu.VMEM((NG, S, 128), jnp.bfloat16),
            pltpu.VMEM((S, D), jnp.float32),
            pltpu.VMEM((H * HP, D), jnp.float32),
            pltpu.VMEM((D, F), jnp.bfloat16),
            pltpu.VMEM((D, F), jnp.bfloat16),
            pltpu.VMEM((F, D), jnp.bfloat16),
            pltpu.SemaphoreType.DMA((3,)),
        ],
        compiler_params=pltpu.CompilerParams(vmem_limit_bytes=100 * 1024 * 1024),
    )(x, wqkv, wo, wr, B_w_gate, B_w_up, B_w_down)
    return out.reshape(1, S, D)
```

```python
import jax
import jax.numpy as jnp
import jax.experimental.pallas as pl
import jax.experimental.pallas.tpu as pltpu

S = 2048
D = 640
H = 32
DH = 20
HP = 32
NG = H * HP // 128
F = 1536
TQ = 512
RV = 128
CT = 512
RC = 256
EPS = 1e-5
ONES_LANE = DH


def _ln(x):
    m = jnp.mean(x, axis=-1, keepdims=True)
    xc = x - m
    v = jnp.mean(xc * xc, axis=-1, keepdims=True)
    return xc * jax.lax.rsqrt(v + EPS)


def _kernel(x_ref, wqkv_ref, wo_ref, wr_ref, wg_hbm, wu_hbm, wd_hbm, o_ref,
            q_s, kT_s, v_s, on_s, lnh_s, wop_s, wg_ref, wu_ref, wd_ref, sems):
    f32 = jnp.float32
    bf16 = jnp.bfloat16
    scale = DH ** -0.5

    lane128 = jax.lax.broadcasted_iota(jnp.int32, (1, 128), 1)
    ones_mask = (lane128 % HP) == ONES_LANE

    cps = [pltpu.make_async_copy(wg_hbm, wg_ref, sems.at[0]),
           pltpu.make_async_copy(wu_hbm, wu_ref, sems.at[1]),
           pltpu.make_async_copy(wd_hbm, wd_ref, sems.at[2])]
    for cp in cps:
        cp.start()

    for hh in range(H):
        wop_s[hh * HP:hh * HP + DH, :] = wo_ref[hh * DH:(hh + 1) * DH, :].astype(f32)
        wop_s[hh * HP + DH:(hh + 1) * HP, :] = jnp.zeros((HP - DH, D), f32)

    zpad_l = jnp.zeros((RC, HP - DH), f32)
    lane_p = jax.lax.broadcasted_iota(jnp.int32, (RC, HP - DH), 1)
    one_pad = jnp.where(lane_p == 0, 1.0, 0.0).astype(f32)
    zpad_r = jnp.zeros((HP - DH, RC), f32)

    def p1(c, carry):
        r0 = pl.multiple_of(c * RC, RC)
        xs = x_ref[pl.ds(r0, RC), :].astype(f32)
        ln = _ln(xs).astype(bf16)
        q = jnp.dot(ln, wqkv_ref[:, 0:D], preferred_element_type=f32) * scale
        k = jnp.dot(ln, wqkv_ref[:, D:2 * D], preferred_element_type=f32)
        v = jnp.dot(ln, wqkv_ref[:, 2 * D:3 * D], preferred_element_type=f32)
        kt = k.T
        for g in range(NG):
            qp, kp, vp = [], [], []
            for j in range(4):
                hh = g * 4 + j
                qp += [q[:, hh * DH:(hh + 1) * DH], zpad_l]
                vp += [v[:, hh * DH:(hh + 1) * DH], one_pad]
                kp += [kt[hh * DH:(hh + 1) * DH, :], zpad_r]
            q_s[g, pl.ds(r0, RC), :] = jnp.concatenate(qp, axis=1).astype(bf16)
            v_s[g, pl.ds(r0, RC), :] = jnp.concatenate(vp, axis=1).astype(bf16)
            kT_s[g, :, pl.ds(r0, RC)] = jnp.concatenate(kp, axis=0).astype(bf16)
        return carry

    with jax.named_scope('p1'):
        jax.lax.fori_loop(0, S // RC, p1, 0)

    er = jax.lax.broadcasted_iota(jnp.int32, (128, 128), 0)
    ec = jax.lax.broadcasted_iota(jnp.int32, (128, 128), 1)
    E = jnp.where((er % HP == ONES_LANE) & (er // HP == ec // HP), 1.0, 0.0).astype(f32)

    def p2(i, carry):
        qb = i // NG
        g = i % NG
        r0 = pl.multiple_of(qb * TQ, TQ)
        qg = q_s[g, pl.ds(r0, TQ), :]
        kT = kT_s[g]
        vg = v_s[g]
        RM = TQ - RV
        qv = qg[RM:, :].astype(f32)
        acc_v = jnp.zeros((RV, 128), f32)
        acc = jnp.zeros((RM, 128), f32)
        for j in range(4):
            hmask = (lane128 // HP) == j
            qm = jnp.where(hmask, qg[:RM], jnp.zeros((RM, 128), bf16))
            s = jnp.dot(qm, kT, preferred_element_type=f32)
            m = jnp.max(s, axis=-1, keepdims=True)
            p = jnp.exp(s - m).astype(bf16)
            o = jnp.dot(p, vg, preferred_element_type=f32)
            acc = jnp.where(hmask, o, acc)
            kf = kT[j * HP:j * HP + 24, :].astype(f32)
            rows = []
            for rb in range(RV // 8):
                q8 = qv[rb * 8:(rb + 1) * 8, :]
                qc = [q8[:, j * HP + d:j * HP + d + 1] for d in range(DH)]
                tiles = []
                for cb in range(S // CT):
                    t = qc[0] * kf[0:1, cb * CT:(cb + 1) * CT]
                    for d in range(1, DH):
                        t = t + qc[d] * kf[d:d + 1, cb * CT:(cb + 1) * CT]
                    tiles.append(t)
                rows.append(jnp.concatenate(tiles, axis=1))
            sv = jnp.concatenate(rows, axis=0)
            mv = jnp.max(sv, axis=-1, keepdims=True)
            pv = jnp.exp(sv - mv).astype(bf16)
            ov = jnp.dot(pv, vg, preferred_element_type=f32)
            acc_v = jnp.where(hmask, ov, acc_v)
        acc = jnp.concatenate([acc, acc_v], axis=0)
        l = jnp.dot(acc, E, preferred_element_type=f32, precision=jax.lax.Precision.HIGHEST)
        on_s[g, pl.ds(r0, TQ), :] = (acc / l).astype(bf16)
        return carry

    with jax.named_scope('p2'):
        jax.lax.fori_loop(0, (S // TQ) * NG, p2, 0)

    wr = wr_ref[...].astype(f32)

    def p3(c, carry):
        best_v, best_i = carry
        r0 = pl.multiple_of(c * RC, RC)
        a = jnp.zeros((RC, D), f32)
        for g in range(NG):
            a = a + jnp.dot(on_s[g, pl.ds(r0, RC), :], wop_s[g * 128:(g + 1) * 128, :].astype(bf16),
                            preferred_element_type=f32)
        a = a.astype(bf16).astype(f32)
        xs = x_ref[pl.ds(r0, RC), :].astype(f32)
        h = (xs + a).astype(bf16).astype(f32)
        lnh = _ln(h).astype(bf16).astype(f32)
        lnh_s[pl.ds(r0, RC), :] = lnh
        o_ref[pl.ds(r0, RC), :] = (h + lnh).astype(o_ref.dtype)
        r = jnp.sum(lnh * wr, axis=-1, keepdims=True)
        r = r.astype(bf16).astype(f32)
        cm = jnp.max(r)
        rows = jax.lax.broadcasted_iota(jnp.int32, (RC, 1), 0) + c * RC
        ci = jnp.min(jnp.where(r == cm, rows, S))
        better = cm > best_v
        return jnp.where(better, cm, best_v), jnp.where(better, ci, best_i)

    with jax.named_scope('p3'):
        best_v, best_i = jax.lax.fori_loop(
            0, S // RC, p3, (jnp.float32(-jnp.inf), jnp.int32(0)))

    for cp in cps:
        cp.wait()
    xsel = lnh_s[pl.ds(best_i, 1), :]
    xsel8 = jnp.broadcast_to(xsel, (8, D)).astype(bf16)
    gt = jnp.dot(xsel8, wg_ref[...], preferred_element_type=f32)
    gt = gt.astype(bf16).astype(f32)
    gt = (gt * jax.nn.sigmoid(gt)).astype(bf16).astype(f32)
    u = jnp.dot(xsel8, wu_ref[...], preferred_element_type=f32).astype(bf16).astype(f32)
    gu = (gt * u).astype(bf16)
    y = jnp.dot(gu, wd_ref[...], preferred_element_type=f32).astype(bf16).astype(f32)
    rs = jax.nn.sigmoid(best_v).astype(bf16).astype(f32)
    y = (y * rs).astype(bf16).astype(f32)
    t0 = pl.multiple_of((best_i // 16) * 16, 16)
    rows = jax.lax.broadcasted_iota(jnp.int32, (16, 1), 0) + t0
    cur = o_ref[pl.ds(t0, 16), :].astype(f32)
    y16 = jnp.broadcast_to(y[0:1, :], (16, D))
    o_ref[pl.ds(t0, 16), :] = jnp.where(rows == best_i, cur + y16, cur).astype(o_ref.dtype)


@jax.jit
def pallas_sequential_preLN__mha_block__moe_arch_mod__prompt_kernel(
    A_x: jax.Array,
    A_wqkv: jax.Array,
    A_wo: jax.Array,
    B_x: jax.Array,
    B_w_r: jax.Array,
    B_w_gate: jax.Array,
    B_w_up: jax.Array,
    B_w_down: jax.Array,
):
    del B_x
    x = A_x.reshape(S, D)
    wqkv = A_wqkv
    wo = A_wo
    wr = B_w_r.reshape(1, D)

    vm = pl.BlockSpec(memory_space=pltpu.VMEM)
    out = pl.pallas_call(
        _kernel,
        out_shape=jax.ShapeDtypeStruct((S, D), A_x.dtype),
        in_specs=[vm] * 4 + [pl.BlockSpec(memory_space=pl.ANY)] * 3,
        out_specs=vm,
        scratch_shapes=[
            pltpu.VMEM((NG, S, 128), jnp.bfloat16),
            pltpu.VMEM((NG, 128, S), jnp.bfloat16),
            pltpu.VMEM((NG, S, 128), jnp.bfloat16),
            pltpu.VMEM((NG, S, 128), jnp.bfloat16),
            pltpu.VMEM((S, D), jnp.float32),
            pltpu.VMEM((H * HP, D), jnp.float32),
            pltpu.VMEM((D, F), jnp.bfloat16),
            pltpu.VMEM((D, F), jnp.bfloat16),
            pltpu.VMEM((F, D), jnp.bfloat16),
            pltpu.SemaphoreType.DMA((3,)),
        ],
        compiler_params=pltpu.CompilerParams(vmem_limit_bytes=100 * 1024 * 1024),
    )(x, wqkv, wo, wr, B_w_gate, B_w_up, B_w_down)
    return out.reshape(1, S, D)
```

```python
import jax
import jax.numpy as jnp
import jax.experimental.pallas as pl
import jax.experimental.pallas.tpu as pltpu

S = 2048
D = 640
H = 32
DH = 20
HP = 32
NG = H * HP // 128
F = 1536
TQ = 1024
RC = 256
EPS = 1e-5
ONES_LANE = DH


def _ln(x):
    m = jnp.mean(x, axis=-1, keepdims=True)
    xc = x - m
    v = jnp.mean(xc * xc, axis=-1, keepdims=True)
    return xc * jax.lax.rsqrt(v + EPS)


def _kernel(x_ref, wqkv_ref, wo_ref, wr_ref, wg_hbm, wu_hbm, wd_hbm, o_ref,
            q_s, kT_s, v_s, on_s, lnh_s, wop_s, wg_ref, wu_ref, wd_ref, sems):
    f32 = jnp.float32
    bf16 = jnp.bfloat16
    scale = DH ** -0.5

    lane128 = jax.lax.broadcasted_iota(jnp.int32, (1, 128), 1)
    ones_mask = (lane128 % HP) == ONES_LANE

    cps = [pltpu.make_async_copy(wg_hbm, wg_ref, sems.at[0]),
           pltpu.make_async_copy(wu_hbm, wu_ref, sems.at[1]),
           pltpu.make_async_copy(wd_hbm, wd_ref, sems.at[2])]
    for cp in cps:
        cp.start()

    for hh in range(H):
        wop_s[hh * HP:hh * HP + DH, :] = wo_ref[hh * DH:(hh + 1) * DH, :].astype(f32)
        wop_s[hh * HP + DH:(hh + 1) * HP, :] = jnp.zeros((HP - DH, D), f32)

    zpad_l = jnp.zeros((RC, HP - DH), f32)
    lane_p = jax.lax.broadcasted_iota(jnp.int32, (RC, HP - DH), 1)
    one_pad = jnp.where(lane_p == 0, 1.0, 0.0).astype(f32)
    zpad_r = jnp.zeros((HP - DH, RC), f32)

    def p1(c, carry):
        r0 = pl.multiple_of(c * RC, RC)
        xs = x_ref[pl.ds(r0, RC), :].astype(f32)
        ln = _ln(xs).astype(bf16)
        q = jnp.dot(ln, wqkv_ref[:, 0:D], preferred_element_type=f32) * scale
        k = jnp.dot(ln, wqkv_ref[:, D:2 * D], preferred_element_type=f32)
        v = jnp.dot(ln, wqkv_ref[:, 2 * D:3 * D], preferred_element_type=f32)
        kt = k.T
        for g in range(NG):
            qp, kp, vp = [], [], []
            for j in range(4):
                hh = g * 4 + j
                qp += [q[:, hh * DH:(hh + 1) * DH], zpad_l]
                vp += [v[:, hh * DH:(hh + 1) * DH], one_pad]
                kp += [kt[hh * DH:(hh + 1) * DH, :], zpad_r]
            q_s[g, pl.ds(r0, RC), :] = jnp.concatenate(qp, axis=1).astype(bf16)
            v_s[g, pl.ds(r0, RC), :] = jnp.concatenate(vp, axis=1).astype(bf16)
            kT_s[g, :, pl.ds(r0, RC)] = jnp.concatenate(kp, axis=0).astype(bf16)
        return carry

    with jax.named_scope('p1'):
        jax.lax.fori_loop(0, S // RC, p1, 0)

    er = jax.lax.broadcasted_iota(jnp.int32, (128, 128), 0)
    ec = jax.lax.broadcasted_iota(jnp.int32, (128, 128), 1)
    E = jnp.where((er % HP == ONES_LANE) & (er // HP == ec // HP), 1.0, 0.0).astype(f32)

    def p2(i, carry):
        qb = i // NG
        g = i % NG
        r0 = pl.multiple_of(qb * TQ, TQ)
        qg = q_s[g, pl.ds(r0, TQ), :]
        kT = kT_s[g]
        vg = v_s[g]
        acc = jnp.zeros((TQ, 128), f32)
        for j in range(4):
            hmask = (lane128 // HP) == j
            qm = jnp.where(hmask, qg, jnp.zeros_like(qg))
            s = jnp.dot(qm, kT, preferred_element_type=f32)
            m = jnp.max(s, axis=-1, keepdims=True)
            p = jnp.exp(s - m).astype(bf16)
            o = jnp.dot(p, vg, preferred_element_type=f32)
            acc = jnp.where(hmask, o, acc)
        l = jnp.dot(acc, E, preferred_element_type=f32, precision=jax.lax.Precision.HIGHEST)
        on_s[g, pl.ds(r0, TQ), :] = (acc / l).astype(bf16)
        return carry

    with jax.named_scope('p2'):
        jax.lax.fori_loop(0, (S // TQ) * NG, p2, 0)

    wr = wr_ref[...].astype(f32)

    def p3(c, carry):
        best_v, best_i = carry
        r0 = pl.multiple_of(c * RC, RC)
        a = jnp.zeros((RC, D), f32)
        for g in range(NG):
            a = a + jnp.dot(on_s[g, pl.ds(r0, RC), :], wop_s[g * 128:(g + 1) * 128, :].astype(bf16),
                            preferred_element_type=f32)
        a = a.astype(bf16).astype(f32)
        xs = x_ref[pl.ds(r0, RC), :].astype(f32)
        h = (xs + a).astype(bf16).astype(f32)
        lnh = _ln(h).astype(bf16).astype(f32)
        lnh_s[pl.ds(r0, RC), :] = lnh
        o_ref[pl.ds(r0, RC), :] = (h + lnh).astype(o_ref.dtype)
        r = jnp.sum(lnh * wr, axis=-1, keepdims=True)
        r = r.astype(bf16).astype(f32)
        cm = jnp.max(r)
        rows = jax.lax.broadcasted_iota(jnp.int32, (RC, 1), 0) + c * RC
        ci = jnp.min(jnp.where(r == cm, rows, S))
        better = cm > best_v
        return jnp.where(better, cm, best_v), jnp.where(better, ci, best_i)

    with jax.named_scope('p3'):
        best_v, best_i = jax.lax.fori_loop(
            0, S // RC, p3, (jnp.float32(-jnp.inf), jnp.int32(0)))

    for cp in cps:
        cp.wait()
    xsel = lnh_s[pl.ds(best_i, 1), :]
    xsel8 = jnp.broadcast_to(xsel, (8, D)).astype(bf16)
    gt = jnp.dot(xsel8, wg_ref[...], preferred_element_type=f32)
    gt = gt.astype(bf16).astype(f32)
    gt = (gt * jax.nn.sigmoid(gt)).astype(bf16).astype(f32)
    u = jnp.dot(xsel8, wu_ref[...], preferred_element_type=f32).astype(bf16).astype(f32)
    gu = (gt * u).astype(bf16)
    y = jnp.dot(gu, wd_ref[...], preferred_element_type=f32).astype(bf16).astype(f32)
    rs = jax.nn.sigmoid(best_v).astype(bf16).astype(f32)
    y = (y * rs).astype(bf16).astype(f32)
    t0 = pl.multiple_of((best_i // 16) * 16, 16)
    rows = jax.lax.broadcasted_iota(jnp.int32, (16, 1), 0) + t0
    cur = o_ref[pl.ds(t0, 16), :].astype(f32)
    y16 = jnp.broadcast_to(y[0:1, :], (16, D))
    o_ref[pl.ds(t0, 16), :] = jnp.where(rows == best_i, cur + y16, cur).astype(o_ref.dtype)


@jax.jit
def pallas_sequential_preLN__mha_block__moe_arch_mod__prompt_kernel(
    A_x: jax.Array,
    A_wqkv: jax.Array,
    A_wo: jax.Array,
    B_x: jax.Array,
    B_w_r: jax.Array,
    B_w_gate: jax.Array,
    B_w_up: jax.Array,
    B_w_down: jax.Array,
):
    del B_x
    x = A_x.reshape(S, D)
    wqkv = A_wqkv
    wo = A_wo
    wr = B_w_r.reshape(1, D)

    vm = pl.BlockSpec(memory_space=pltpu.VMEM)
    out = pl.pallas_call(
        _kernel,
        out_shape=jax.ShapeDtypeStruct((S, D), A_x.dtype),
        in_specs=[vm] * 4 + [pl.BlockSpec(memory_space=pl.ANY)] * 3,
        out_specs=vm,
        scratch_shapes=[
            pltpu.VMEM((NG, S, 128), jnp.bfloat16),
            pltpu.VMEM((NG, 128, S), jnp.bfloat16),
            pltpu.VMEM((NG, S, 128), jnp.bfloat16),
            pltpu.VMEM((NG, S, 128), jnp.bfloat16),
            pltpu.VMEM((S, D), jnp.float32),
            pltpu.VMEM((H * HP, D), jnp.float32),
            pltpu.VMEM((D, F), jnp.bfloat16),
            pltpu.VMEM((D, F), jnp.bfloat16),
            pltpu.VMEM((F, D), jnp.bfloat16),
            pltpu.SemaphoreType.DMA((3,)),
        ],
        compiler_params=pltpu.CompilerParams(vmem_limit_bytes=100 * 1024 * 1024),
    )(x, wqkv, wo, wr, B_w_gate, B_w_up, B_w_down)
    return out.reshape(1, S, D)
```
